```python
import os as _os
_os.environ.setdefault("JAX_PLATFORMS", "cpu")
import jax
import jax.numpy as jnp

def _softmax(x, axis=-1):
    return jax.nn.softmax(x, axis=axis)
def _gelu(x):
    return jax.nn.gelu(x, approximate=True)
def _silu(x):
    return jax.nn.silu(x)
def _sigmoid(x):
    return jax.nn.sigmoid(x)
def _layernorm(x, axis=-1, eps=1e-5):
    m = jnp.mean(x, axis=axis, keepdims=True)
    v = jnp.var(x, axis=axis, keepdims=True)
    return (x - m) / jnp.sqrt(v + eps)
def _scatter_add(tgt, idx, src, axis=0):
    return tgt.at[idx].add(src)
def _segment_sum(src, seg, n):
    return jax.ops.segment_sum(src, seg, n)
class _Rng:
    def __init__(self, key):
        self._k = key
    def _next(self):
        self._k, sub = jax.random.split(self._k)
        return sub
    def normal(self, shape):
        return jax.random.normal(self._next(), shape, dtype=jnp.bfloat16)
    def randint(self, lo, hi, shape):
        return jax.random.randint(self._next(), shape, lo, hi, dtype=jnp.int32)
    def uniform(self, shape, lo=0.0, hi=1.0):
        return jax.random.uniform(self._next(), shape, jnp.bfloat16, lo, hi)
    def permutation(self, n):
        return jax.random.permutation(self._next(), n)


kernel_name = 'gated_mix__softmax_full_mha__dense_activation_relu__prompt'

def setup_inputs():
    _rng = _Rng(jax.random.key(int.from_bytes(__import__("os").urandom(4), "little")))
    _w = (lambda a: (lambda t: t.astype(jnp.bfloat16) if jnp.issubdtype(t.dtype, jnp.floating) else t)(jnp.asarray(a)))
    def _A_setup():
        B, S, D = 1, 2048, 640
        return {
            "x": _w((lambda *s: _rng.normal(s) * 0.05)(B, S, D)),
            "wqkv": _w((lambda *s: _rng.normal(s) * 0.8)(D, 3 * D)),
            "wo": _w((lambda *s: _rng.normal(s) * 0.05)(D, D)),
        }
    _A_in = _A_setup()

    def _B_setup():
        B, S, D, Dff = 1, 2048, 640, 1536
        return {
            "x": _w((lambda *s: _rng.normal(s) * 0.05)(B, S, D)),
            "w1": _w((lambda *s: _rng.normal(s) * 0.05)(D, Dff)),
            "w2": _w((lambda *s: _rng.normal(s) * 0.05)(Dff, D)),
        }
    _B_in = _B_setup()

    return {
        "A_x": _A_in["x"],
        "A_wqkv": _A_in["wqkv"],
        "A_wo": _A_in["wo"],
        "B_x": _B_in["x"],
        "B_w1": _B_in["w1"],
        "B_w2": _B_in["w2"],
        "gate_w": _w((lambda *s: _rng.normal(s) * 0.05)(640) * 16.0),
    }

def reference(A_x, A_wqkv, A_wo, B_x, B_w1, B_w2, gate_w):
    def _A_ref(x, wqkv, wo):
        B, S, D = x.shape
        H = 32; Dh = D // H
        qkv = (lambda x, *d: x.transpose(*d))((x @ wqkv).reshape(B, S, 3, H, Dh), 2, 0, 3, 1, 4)
        q, k, v = qkv[0], qkv[1], qkv[2]
        scale = Dh ** -0.5
        scores = jnp.einsum("bhqd,bhkd->bhqk", q, k) * scale
        p = _softmax(scores, axis=-1)
        o = jnp.einsum("bhqk,bhkd->bhqd", p, v)
        return (lambda x, *d: x.transpose(*d))(o, 0, 2, 1, 3).reshape(B, S, D) @ wo

    def _B_ref(x, w1, w2):
        h = jnp.einsum("bsd,df->bsf", x, w1)
        zero = jnp.zeros_like(h)
        h = jnp.maximum(h, zero)
        return jnp.einsum("bsf,fd->bsd", h, w2)

    x = A_x
    g = _sigmoid((x * gate_w).sum(-1, keepdims=True))
    a = _A_ref(x, A_wqkv, A_wo)
    b = _B_ref(x, B_w1, B_w2)
    return g * a + (1 - g) * b
```

```python
import math
import functools

import jax
import jax.numpy as jnp
from jax import lax
import jax.experimental.pallas as pl
import jax.experimental.pallas.tpu as pltpu

H = 32
LANES = 128
BF16 = jnp.bfloat16
F32 = jnp.float32


def _kernel(x_hbm, wqkv_hbm, wo_hbm, w1_hbm, w2_hbm, gw_ref, o_hbm,
            x_s, wqkv_s, wo_s, w1_s, w2_s, k_s, qt_s, vt_s, ot_s, b_s, o_s,
            xsem, wsem, osem, *, S, D, TQ, NH, SK, FP):
    Dh = D // H
    nt = D // LANES
    nq = S // TQ
    ng = H // NH
    FR = TQ // ng
    qscale = (Dh ** -0.5) * math.log2(math.e)
    tn = (((0,), (1,)), ((), ()))

    def x_copy(c):
        rows = pl.ds(pl.multiple_of(c * TQ, TQ), TQ)
        return pltpu.make_async_copy(x_hbm.at[rows, :], x_s.at[rows, :], xsem.at[c])

    def wqkv_copy(j):
        return pltpu.make_async_copy(wqkv_hbm.at[:, pl.ds(j * D, D)], wqkv_s.at[j], wsem.at[j])

    w1_copy = pltpu.make_async_copy(w1_hbm, w1_s, wsem.at[3])
    w2_copy = pltpu.make_async_copy(w2_hbm, w2_s, wsem.at[4])
    wo_copy = pltpu.make_async_copy(wo_hbm, wo_s, wsem.at[5])

    def o_copy(c):
        rows = pl.ds(pl.multiple_of(c * TQ, TQ), TQ)
        return pltpu.make_async_copy(o_s.at[rows, :], o_hbm.at[rows, :], osem.at[c])

    x_copy(0).start()
    wqkv_copy(1).start()
    wqkv_copy(0).start()
    wqkv_copy(2).start()
    for c in range(1, nq):
        x_copy(c).start()
    w1_copy.start()
    w2_copy.start()
    wo_copy.start()

    def project(c, carry):
        rows = pl.ds(pl.multiple_of(c * TQ, TQ), TQ)
        x_copy(c).wait()

        @pl.when(c == 0)
        def _():
            wqkv_copy(1).wait()

        xc = x_s[rows, :]
        k = jnp.dot(xc, wqkv_s[1], preferred_element_type=F32)
        hi = lax.broadcasted_iota(jnp.int32, (TQ, LANES), 1) >= LANES // 2
        for t in range(nt):
            kt = k[:, t * LANES:(t + 1) * LANES]
            k_s[t, rows, :] = kt.astype(BF16)
            if t + 1 < nt:
                kn = k[:, (t + 1) * LANES:(t + 2) * LANES]
                k_s[nt + t, rows, :] = jnp.where(hi, kt, kn).astype(BF16)

        @pl.when(c == 0)
        def _():
            wqkv_copy(0).wait()
            wqkv_copy(2).wait()

        xc = x_s[rows, :]
        qt = lax.dot_general(wqkv_s[0], xc, tn, preferred_element_type=F32)
        qt_s[c] = (qt * qscale).astype(BF16)
        vt = lax.dot_general(wqkv_s[2], xc, tn, preferred_element_type=F32)
        vt_s[c] = vt.astype(BF16).astype(F32)
        return carry

    lax.fori_loop(0, nq, project, 0)
    w1_copy.wait()
    w2_copy.wait()
    wo_copy.wait()

    CH = LANES
    n = S // CH
    cpb = TQ // CH

    def heads(i, qi):
        h0 = i * NH
        prow = lax.broadcasted_iota(jnp.int32, (LANES // 2, TQ), 0) * 2
        row8 = lax.broadcasted_iota(jnp.int32, (8, CH), 0)

        def prep(j):
            lo = (h0 + j) * Dh
            ta = lo // LANES
            tb = (lo + Dh - 1) // LANES
            ra = pl.multiple_of(ta * LANES, LANES)
            rb = pl.multiple_of(tb * LANES, LANES)
            qa = pltpu.bitcast(qt_s[qi, pl.ds(ra, LANES), :], jnp.uint32)
            qb = pltpu.bitcast(qt_s[qi, pl.ds(rb, LANES), :], jnp.uint32)
            da = prow + (ra - lo)
            db = prow + (rb - lo)
            ma = (da >= 0) & (da < Dh)
            mb = (db >= 0) & (db < Dh)
            q = jnp.where(ma, qa, jnp.where(mb, qb, jnp.zeros_like(qb)))
            kt = jnp.where(ta == tb, ta, nt + ta)
            v0 = pl.multiple_of(lo - (4 if j % 2 else 0), 8)
            return pltpu.bitcast(q, BF16), kt, v0

        def ffn1():
            r0 = pl.multiple_of(qi * TQ + i * FR, FR)
            hid = jnp.dot(x_s[pl.ds(r0, FR), :], w1_s[...], preferred_element_type=F32)
            return jnp.maximum(hid, 0.0).astype(BF16)

        def ffn2(hid):
            b_s[pl.ds(pl.multiple_of(i * FR, FR), FR), :] = jnp.dot(
                hid, w2_s[...], preferred_element_type=F32)

        hid = ffn1()
        if FP == 0:
            ffn2(hid)
        hp = [prep(j) for j in range(NH)]
        pend = {}
        accs = [None] * NH
        outs = [None] * NH
        m = None
        for t in range(NH * n + SK):
            if t < NH * n:
                j, c = divmod(t, n)
                q, kt, _ = hp[j]
                s = jnp.dot(k_s[kt, pl.ds(c * CH, CH), :], q, preferred_element_type=F32)
                mc = jnp.max(jnp.max(s.reshape(CH // 8, 8, TQ), axis=0), axis=0, keepdims=True)
                if c == 0:
                    alpha = None
                    m = mc
                else:
                    mn = jnp.maximum(m, mc)
                    alpha = jnp.exp2(m - mn)
                    m = mn
                pend[t] = (jnp.exp2(s - m).astype(BF16), alpha)
            if FP == 1 and t == NH * n:
                ffn2(hid)
            if t >= SK:
                j, c = divmod(t - SK, n)
                p, alpha = pend.pop(t - SK)
                v0 = hp[j][2]
                blk = c // cpb
                cols = pl.ds((c % cpb) * CH, CH)
                if j % 2 == 0:
                    v = jnp.concatenate([
                        vt_s[blk, pl.ds(v0, 16), cols],
                        jnp.where(row8 < 4, vt_s[blk, pl.ds(v0 + 16, 8), cols], 1.0)], axis=0)
                else:
                    v = jnp.concatenate([
                        jnp.where(row8 >= 4, vt_s[blk, pl.ds(v0, 8), cols], 1.0),
                        vt_s[blk, pl.ds(v0 + 8, 16), cols]], axis=0)
                o = jnp.dot(v, p, preferred_element_type=F32)
                accs[j] = o if c == 0 else accs[j] * alpha + o
                if c == n - 1:
                    a = accs[j]
                    l = a[20:21] if j % 2 == 0 else a[0:1]
                    outs[j] = a * (1.0 / l)
                    if j % 4 == 3:
                        r8 = lax.broadcasted_iota(jnp.int32, (8, TQ), 0)
                        parts = []
                        for e in (j - 3, j - 1):
                            oe, oo = outs[e], outs[e + 1]
                            parts += [oe[0:16], jnp.where(r8 < 4, oe[16:24], oo[0:8]), oo[8:24]]
                        r0 = pl.multiple_of((h0 + j - 3) * Dh, 16)
                        ot_s[pl.ds(r0, 4 * Dh), :] = jnp.concatenate(parts, axis=0).astype(BF16)
        return qi

    def qblock(qi, carry):
        lax.fori_loop(0, ng, heads, qi)
        rows = pl.ds(pl.multiple_of(qi * TQ, TQ), TQ)
        a = lax.dot_general(ot_s[...], wo_s[...], (((0,), (0,)), ((), ())),
                            preferred_element_type=F32)
        gw = gw_ref[...].astype(F32).reshape(1, D)
        z = jnp.sum(x_s[rows, :].astype(F32) * gw, axis=-1, keepdims=True)
        g = jax.nn.sigmoid(z)
        o_s[rows, :] = (g * a + (1.0 - g) * b_s[...]).astype(o_s.dtype)
        o_copy(qi).start()
        return carry

    lax.fori_loop(0, nq, qblock, 0)
    for c in range(nq):
        o_copy(c).wait()


TQ, NH, SK, FP = 512, 8, 2, 1


@jax.jit
def pallas_gated_mix__softmax_full_mha__dense_activation_relu__prompt_kernel(A_x, A_wqkv, A_wo, B_x, B_w1, B_w2, gate_w):
    del B_x
    B, S, D = A_x.shape
    Dff = B_w1.shape[1]
    nt = D // LANES
    nq = S // TQ
    hbm = pl.BlockSpec(memory_space=pl.ANY)
    out = pl.pallas_call(
        functools.partial(_kernel, S=S, D=D, TQ=TQ, NH=NH, SK=SK, FP=FP),
        in_specs=[hbm] * 5 + [pl.BlockSpec(memory_space=pltpu.VMEM)],
        out_specs=hbm,
        out_shape=jax.ShapeDtypeStruct((S, D), A_x.dtype),
        scratch_shapes=[
            pltpu.VMEM((S, D), BF16),
            pltpu.VMEM((3, D, D), BF16),
            pltpu.VMEM((D, D), BF16),
            pltpu.VMEM((D, Dff), BF16),
            pltpu.VMEM((Dff, D), BF16),
            pltpu.VMEM((2 * nt - 1, S, LANES), BF16),
            pltpu.VMEM((nq, D, TQ), BF16),
            pltpu.VMEM((nq, D, TQ), F32),
            pltpu.VMEM((D, TQ), BF16),
            pltpu.VMEM((TQ, D), F32),
            pltpu.VMEM((S, D), A_x.dtype),
            pltpu.SemaphoreType.DMA((nq,)),
            pltpu.SemaphoreType.DMA((6,)),
            pltpu.SemaphoreType.DMA((nq,)),
        ],
        compiler_params=pltpu.CompilerParams(
            vmem_limit_bytes=100 * 2**20),
        name="gmk",
    )(A_x.reshape(S, D), A_wqkv, A_wo, B_w1, B_w2, gate_w)
    return out.reshape(B, S, D)
```

```python
import math

import jax
import jax.numpy as jnp
from jax import lax
import jax.experimental.pallas as pl
import jax.experimental.pallas.tpu as pltpu

H = 32
LANES = 128
SUB = 8
TQ = 512
CH = 128
G = 8
NH = 8
SKEW = 2
VR = 24
FFN_OUT = 4
NO = 2
SPLIT = 40

BF16 = jnp.bfloat16
F32 = jnp.float32
U32 = jnp.uint32


def _tree_sum(ts):
    while len(ts) > 1:
        ts = [ts[a] + ts[a + 1] if a + 1 < len(ts) else ts[a] for a in range(0, len(ts), 2)]
    return ts[0]


def _kernel(x_hbm, wqkv_hbm, wo_hbm, w1_hbm, w2_hbm, gw_hbm, o_hbm,
            x_s, wqkv_s, wt_s, wo_s, w1_s, w2_s, k_s, kb_s, qf_s, qm_s, vt_s, h_s, ot_s, b_s,
            o_s, gw_s, m_s, xsem, wsem, osem):
    S, D = x_s.shape
    Dff = w1_s.shape[1]
    Dh = D // H
    nt = D // LANES
    nq = S // TQ
    ng = H // NH
    n = S // CH
    cpb = TQ // CH
    GR = NH * Dh
    FR = TQ // ng
    OR = TQ // NO
    half = LANES // 2
    qscale = (Dh ** -0.5) * math.log2(math.e)
    nt_dims = (((1,), (1,)), ((), ()))
    tn_dims = (((0,), (0,)), ((), ()))

    def block(c, size):
        return pl.ds(pl.multiple_of(c * size, size), size)

    def x_copy(c):
        rows = block(c, TQ)
        return pltpu.make_async_copy(x_hbm.at[rows, :], x_s.at[rows, :], xsem.at[c])

    def wqkv_copy(j):
        return pltpu.make_async_copy(wqkv_hbm.at[:, pl.ds(j * D, D)], wqkv_s.at[j], wsem.at[j])

    def o_copy(c):
        rows = block(c, OR)
        return pltpu.make_async_copy(o_s.at[rows, :], o_hbm.at[rows, :], osem.at[c])

    w1_copy = pltpu.make_async_copy(w1_hbm, w1_s, wsem.at[3])
    w2_copy = pltpu.make_async_copy(w2_hbm, w2_s, wsem.at[4])
    wo_copy = pltpu.make_async_copy(wo_hbm, wo_s, wsem.at[5])
    gw_copy = pltpu.make_async_copy(gw_hbm, gw_s, wsem.at[6])

    x_copy(0).start()
    wqkv_copy(1).start()

    def q_vregs(h):
        return range(h * Dh // 2 // SUB, ((h + 1) * Dh // 2 + SUB - 1) // SUB)

    def zero_q(c, carry):
        for h in range(H):
            live = [r * SUB % half for r in q_vregs(h)]
            for r in range(0, half, SUB):
                if r not in live:
                    qm_s[c * H + h, pl.ds(r, SUB), :] = jnp.zeros((SUB, TQ), U32)
        return carry

    lax.fori_loop(0, nq, zero_q, 0)
    x_copy(0).wait()
    wqkv_copy(1).wait()
    for c in range(1, nq):
        x_copy(c).start()
    wqkv_copy(0).start()
    wqkv_copy(2).start()

    def project_k(c):
        rows = block(c, TQ)
        k = jnp.dot(x_s[rows, :], wqkv_s[1], preferred_element_type=F32)
        k = k.astype(BF16).astype(F32)
        upper = lax.broadcasted_iota(jnp.int32, (TQ, LANES), 1) >= half
        for t in range(nt):
            kt = k[:, t * LANES:(t + 1) * LANES]
            k_s[t, rows, :] = kt
            if t + 1 < nt:
                k_s[nt + t, rows, :] = jnp.where(upper, kt, k[:, (t + 1) * LANES:(t + 2) * LANES])

    def k_step(c, carry):
        @pl.when(c > 0)
        def _():
            x_copy(c).wait()

        @pl.when(c == 1)
        def _():
            w1_copy.start()
            w2_copy.start()
            wo_copy.start()
            gw_copy.start()

        project_k(c)
        return carry

    lax.fori_loop(0, nq - 1, k_step, 0)
    x_copy(nq - 1).wait()
    wqkv_copy(0).wait()
    wqkv_copy(2).wait()
    wt_s[0] = wqkv_s[0].T
    wt_s[1] = wqkv_s[2].T
    project_k(nq - 1)
    w1_copy.wait()

    def project(c, carry):
        rows = block(c, TQ)
        sub = lax.broadcasted_iota(jnp.int32, (SUB, TQ), 0)

        def spread(lanes):
            kv = [jnp.concatenate(
                [k_s[t, pl.ds(pl.multiple_of(c * TQ + (u + 1) * CH - G, G), G), :]
                 for u in range(cpb)], axis=0) for t in range(nt)]
            for lane in lanes:
                for t in range(nt):
                    i, r = divmod(t * LANES + lane, GR)
                    w = jnp.broadcast_to(kv[t][:, lane:lane + 1], (cpb * G, LANES))
                    for u in range(cpb):
                        kb_s[i, c * cpb + u, pl.ds(r * G, G), :] = w[u * G:(u + 1) * G]

        spread(range(0, SPLIT))
        xc = x_s[rows, :]
        qt = lax.dot_general(wt_s[0], xc, nt_dims, preferred_element_type=F32)
        qt = (qt * qscale).astype(BF16)
        qf = qt.astype(F32)
        for i in range(ng):
            qf_s[c, i] = qf[i * GR:(i + 1) * GR]
        qw = pltpu.bitcast(qt, U32)
        zero = jnp.zeros((SUB, TQ), U32)
        for h in range(H):
            lo, hi = h * Dh // 2, (h + 1) * Dh // 2
            for r in q_vregs(h):
                w = qw[r * SUB:(r + 1) * SUB]
                if r * SUB < lo:
                    w = jnp.where(sub >= lo - r * SUB, w, zero)
                if (r + 1) * SUB > hi:
                    w = jnp.where(sub < hi - r * SUB, w, zero)
                qm_s[c * H + h, pl.ds(r * SUB % half, SUB), :] = w

        vt = lax.dot_general(wt_s[1], xc, nt_dims, preferred_element_type=F32)
        vt = vt.astype(BF16).astype(F32)
        for h in range(0, H, 2):
            r = h * Dh
            mid = vt[r + 16:r + 24]
            i, j = divmod(h, NH)
            vt_s[i, c, j] = jnp.concatenate(
                [vt[r:r + 16], jnp.where(sub < 4, mid, 1.0)], axis=0)
            vt_s[i, c, j + 1] = jnp.concatenate(
                [jnp.where(sub >= 4, mid, 1.0), vt[r + 24:r + 40]], axis=0)

        spread(range(SPLIT, LANES))
        hid = jnp.dot(x_s[rows, :], w1_s[...], preferred_element_type=F32)
        h_s[rows, :] = jnp.maximum(hid, 0.0).astype(BF16)
        return carry

    lax.fori_loop(0, nq, project, 0)
    w2_copy.wait()
    wo_copy.wait()
    gw_copy.wait()

    def heads(i, qi):
        h0 = i * NH

        def k_tile(j):
            lo = (h0 + j) * Dh
            first = lo // LANES
            last = (lo + Dh - 1) // LANES
            return jnp.where(first == last, first, nt + first)

        tiles = [k_tile(j) for j in range(NH)]
        pending = {}
        acc = [None] * NH
        out = [None] * NH
        m = None
        for t in range(NH * n + SKEW):
            if t < NH * n:
                j, c = divmod(t, n)
                s = jnp.dot(k_s[tiles[j], pl.ds(c * CH, CH - G), :],
                            pltpu.bitcast(qm_s[qi * H + h0 + j], BF16),
                            preferred_element_type=F32)
                kb = [kb_s[i, c, pl.ds((j * Dh + d) * G, G), :] for d in range(Dh)]
                sv = [_tree_sum([kb[d] * qf_s[qi, i, pl.ds(j * Dh + d, 1), pl.ds(u * LANES, LANES)]
                                 for d in range(Dh)]) for u in range(TQ // LANES)]
                s = jnp.concatenate([s, jnp.concatenate(sv, axis=1)], axis=0)
                mc = jnp.max(s.reshape(CH // SUB, SUB, TQ), axis=0)
                if c == 0:
                    alpha = None
                    m = jnp.max(mc, axis=0, keepdims=True)
                else:
                    m_new = jnp.max(jnp.maximum(mc, m), axis=0, keepdims=True)
                    alpha = jnp.exp2(m - m_new)
                    m = m_new
                m_s[...] = m[:, :LANES]
                pending[t] = (jnp.exp2(s - m).astype(BF16), alpha)
            if t == NH * n:
                cols = pl.ds(FFN_OUT * LANES, Dff - FFN_OUT * LANES)
                b = jnp.dot(h_s[block(qi * ng + i, FR), cols], w2_s[cols, :],
                            preferred_element_type=F32)
            if t >= SKEW:
                j, c = divmod(t - SKEW, n)
                p, alpha = pending.pop(t - SKEW)
                v = vt_s[i, c // cpb, j, :, pl.ds((c % cpb) * CH, CH)]
                o = jnp.dot(v, p, preferred_element_type=F32)
                acc[j] = o if c == 0 else acc[j] * alpha + o
                if c == n - 1:
                    denom = acc[j][Dh:Dh + 1] if j % 2 == 0 else acc[j][0:1]
                    out[j] = acc[j] * (1.0 / denom)
                    if j % 4 == 3:
                        sub = lax.broadcasted_iota(jnp.int32, (SUB, TQ), 0)
                        parts = []
                        for e in (j - 3, j - 1):
                            even, odd = out[e], out[e + 1]
                            parts += [even[0:16], jnp.where(sub < 4, even[16:24], odd[0:8]),
                                      odd[8:24]]
                        r0 = pl.multiple_of((h0 + j - 3) * Dh, 16)
                        ot_s[pl.ds(r0, 4 * Dh), :] = jnp.concatenate(parts, axis=0).astype(BF16)
        b_s[block(i, FR), :] = b
        return qi

    def query_block(qi, carry):
        lax.fori_loop(0, ng, heads, qi)
        gw = gw_s[...].astype(F32).reshape(1, D)
        cols = pl.ds(0, FFN_OUT * LANES)
        for u in range(NO):
            rows = block(qi * NO + u, OR)
            b = b_s[pl.ds(u * OR, OR), :] + jnp.dot(h_s[rows, cols], w2_s[cols, :],
                                                    preferred_element_type=F32)
            a = lax.dot_general(ot_s[:, pl.ds(u * OR, OR)], wo_s[...], tn_dims,
                                preferred_element_type=F32)
            g = jax.nn.sigmoid(jnp.sum(x_s[rows, :].astype(F32) * gw, axis=-1, keepdims=True))
            o_s[rows, :] = (g * a + (1.0 - g) * b).astype(o_s.dtype)
            o_copy(qi * NO + u).start()
        return carry

    lax.fori_loop(0, nq, query_block, 0)
    for c in range(nq * NO):
        o_copy(c).wait()


@jax.jit
def pallas_gated_mix__softmax_full_mha__dense_activation_relu__prompt_kernel(
    A_x: jax.Array,
    A_wqkv: jax.Array,
    A_wo: jax.Array,
    B_x: jax.Array,
    B_w1: jax.Array,
    B_w2: jax.Array,
    gate_w: jax.Array,
):
    del B_x
    B, S, D = A_x.shape
    Dff = B_w1.shape[1]
    assert B == 1 and D == 20 * H and S % TQ == 0 and S // TQ >= 3
    nt = D // LANES
    nq = S // TQ
    ng = H // NH
    hbm = pl.BlockSpec(memory_space=pl.ANY)
    out = pl.pallas_call(
        _kernel,
        in_specs=[hbm] * 6,
        out_specs=hbm,
        out_shape=jax.ShapeDtypeStruct((S, D), A_x.dtype),
        scratch_shapes=[
            pltpu.VMEM((S, D), BF16),
            pltpu.VMEM((3, D, D), BF16),
            pltpu.VMEM((2, D, D), BF16),
            pltpu.VMEM((D, D), BF16),
            pltpu.VMEM((D, Dff), BF16),
            pltpu.VMEM((Dff, D), BF16),
            pltpu.VMEM((2 * nt - 1, S, LANES), F32),
            pltpu.VMEM((ng, S // CH, D // ng * G, LANES), F32),
            pltpu.VMEM((nq, ng, D // ng, TQ), F32),
            pltpu.VMEM((nq * H, LANES // 2, TQ), U32),
            pltpu.VMEM((ng, nq, NH, VR, TQ), F32),
            pltpu.VMEM((S, Dff), BF16),
            pltpu.VMEM((D, TQ), BF16),
            pltpu.VMEM((TQ, D), F32),
            pltpu.VMEM((S, D), A_x.dtype),
            pltpu.VMEM((D,), BF16),
            pltpu.VMEM((1, LANES), F32),
            pltpu.SemaphoreType.DMA((nq,)),
            pltpu.SemaphoreType.DMA((7,)),
            pltpu.SemaphoreType.DMA((nq * NO,)),
        ],
        compiler_params=pltpu.CompilerParams(vmem_limit_bytes=120 * 2**20),
        name="gated_mix_mha_ffn",
    )(A_x.reshape(S, D), A_wqkv, A_wo, B_w1, B_w2, gate_w)
    return out.reshape(B, S, D)
```
